```python
import os as _os
_os.environ.setdefault('JAX_PLATFORMS', 'cpu')
import jax
import jax.numpy as jnp

def _softmax(x, axis=-1):
    return jax.nn.softmax(x, axis=axis)

def _gelu(x):
    return jax.nn.gelu(x, approximate=True)

def _silu(x):
    return jax.nn.silu(x)

def _sigmoid(x):
    return jax.nn.sigmoid(x)

def _layernorm(x, axis=-1, eps=1e-05):
    m = jnp.mean(x, axis=axis, keepdims=True)
    v = jnp.var(x, axis=axis, keepdims=True)
    return (x - m) / jnp.sqrt(v + eps)

def _scatter_add(tgt, idx, src, axis=0):
    return tgt.at[idx].add(src)

def _segment_sum(src, seg, n):
    return jax.ops.segment_sum(src, seg, n)

class _Rng:

    def __init__(self, key):
        self._k = key

    def _next(self):
        self._k, sub = jax.random.split(self._k)
        return sub

    def normal(self, shape):
        return jax.random.normal(self._next(), shape, dtype=jnp.bfloat16)

    def randint(self, lo, hi, shape):
        return jax.random.randint(self._next(), shape, lo, hi, dtype=jnp.int32)

    def uniform(self, shape, lo=0.0, hi=1.0):
        return jax.random.uniform(self._next(), shape, jnp.bfloat16, lo, hi)

    def permutation(self, n):
        return jax.random.permutation(self._next(), n)
kernel_name = 'standalone__conformer_conv_module__speech'

def setup_inputs():
    _rng = _Rng(jax.random.key(int.from_bytes(__import__("os").urandom(4), "little")))
    _w = lambda a: (lambda t: t.astype(jnp.bfloat16) if jnp.issubdtype(t.dtype, jnp.floating) else t)(jnp.asarray(a))
    B, T, D, K = (2, 4000, 512, 15)
    return {'x': _w((lambda *s: _rng.normal(s) * 0.2)(B, T, D)), 'w_pw1': _w((lambda *s: _rng.normal(s) * 0.2)(D, 2 * D)), 'dw': _w((lambda *s: _rng.normal(s) * 0.05)(K, D)), 'w_pw2': _w((lambda *s: _rng.normal(s) * 0.05)(D, D))}

def reference(x, w_pw1, dw, w_pw2):
    B, T, D = x.shape
    K = dw.shape[0]
    h = x @ w_pw1
    a, b = (h[..., :D].copy(), h[..., D:].copy())
    h = a * _sigmoid(b)
    pad = K // 2
    hp = jnp.pad(h, ((0, 0), (pad, pad), (0, 0)))
    out = jnp.zeros_like(h)
    for i in range(K):
        out = out + hp[:, i:i + T, :] * dw[i][None, None, :]
    return _silu(out) @ w_pw2
```

```python
import jax
import jax.numpy as jnp
from jax import lax
import jax.experimental.pallas as pl
import jax.experimental.pallas.tpu as pltpu

P = 688
HS = 400
TAIL = (256, 128)
LAG = 16
ZP = 8
CARRY = 24

def _split(lo, hi, hs, tail=()):
    out = []
    r = lo
    body_end = hi - sum(tail)
    n_tiles = max(1, round((body_end - lo) / hs))
    units = (body_end - lo) // 16
    assert (body_end - lo) % 16 == 0
    for i in range(n_tiles):
        u = units // n_tiles + (1 if i < units % n_tiles else 0)
        out.append((r, r + 16 * u)); r += 16 * u
    for n in tail:
        out.append((r, r + n)); r += n
    assert r == hi
    return out

@jax.jit
def pallas_standalone__conformer_conv_module__speech_kernel(x, w_pw1, dw, w_pw2):
    B, T, D = x.shape
    K = dw.shape[0]
    PAD = K // 2
    NC = D // 128
    KH = D // 2
    f32 = jnp.float32
    bf16 = jnp.bfloat16
    R = B * T
    x2 = x.reshape(R, D)

    tail = TAIL
    mt = _split(P, T, HS, tail)
    mb = [(lo - LAG, (hi - LAG) if hi < T else T) for lo, hi in mt]
    pt = _split(0, P, P // 2)
    pb = [(max(lo - LAG, 0), hi - LAG) for lo, hi in pt]

    W1A = R
    W1B = W1A + D
    W2 = W1B + D
    DW = W2 + D
    AR = DW

    def body(x_hbm, w1_hbm, dw_hbm, w2_hbm, o_hbm, arena, obuf, hp, gp, gm, dwbuf, sem):
        cp = pltpu.make_async_copy
        G1 = [cp(w1_hbm.at[pl.ds(0, KH), pl.ds(0, D)], arena.at[pl.ds(W1A, KH), :], sem.at[0]),
              cp(w1_hbm.at[pl.ds(0, KH), pl.ds(D, D)], arena.at[pl.ds(W1B, KH), :], sem.at[0]),
              cp(x_hbm.at[pl.ds(0, P), pl.ds(0, KH)], arena.at[pl.ds(0, P), pl.ds(0, KH)], sem.at[0])]
        G2 = [cp(w1_hbm.at[pl.ds(KH, KH), pl.ds(0, D)], arena.at[pl.ds(W1A + KH, KH), :], sem.at[1]),
              cp(w1_hbm.at[pl.ds(KH, KH), pl.ds(D, D)], arena.at[pl.ds(W1B + KH, KH), :], sem.at[1]),
              cp(x_hbm.at[pl.ds(0, P), pl.ds(KH, KH)], arena.at[pl.ds(0, P), pl.ds(KH, KH)], sem.at[1]),
              cp(dw_hbm, dwbuf, sem.at[1]),
              cp(w2_hbm, arena.at[pl.ds(W2, D), :], sem.at[1])]
        G3 = [cp(x_hbm.at[pl.ds(T, P), :], arena.at[pl.ds(T, P), :], sem.at[2])]
        def xm(b):
            return cp(x_hbm.at[pl.ds(b * T + P, T - P), :], arena.at[pl.ds(b * T + P, T - P), :], sem.at[3 + b])
        def ocopy(row, n):
            return cp(obuf.at[pl.ds(row, n), :], o_hbm.at[pl.ds(row, n), :], sem.at[5])

        def w1(c, half, klo=0, khi=D):
            base = W1B if half else W1A
            return arena[pl.ds(base + klo, khi - klo), c * 128:(c + 1) * 128]

        def glu(a, b):
            return a * (jnp.tanh(0.5 * b) + 1.0)

        def mm1(xv, gref, grow):
            n = xv.shape[0]
            for c in range(NC):
                a = jnp.dot(xv, w1(c, 0), preferred_element_type=f32)
                b = jnp.dot(xv, w1(c, 1), preferred_element_type=f32)
                gref[c, pl.ds(grow, n), :] = glu(a, b)

        def conv(gref, grow, n, c):
            dwf = dwbuf[:, c * 128:(c + 1) * 128].astype(f32) * 0.25
            acc = None
            for i in range(K):
                term = gref[c, pl.ds(grow - PAD + i, n), :] * dwf[i:i + 1, :]
                acc = term if acc is None else acc + term
            sv = acc * (jnp.tanh(acc) + 1.0)
            return sv.astype(bf16)

        def conv_mm2(gref, grow, n, orow):
            sv = jnp.concatenate([conv(gref, grow, n, c) for c in range(NC)], axis=1)
            obuf[pl.ds(orow, n), :] = jnp.dot(sv, arena[pl.ds(W2, D), :], preferred_element_type=f32).astype(bf16)
            ocopy(orow, n).start()

        for g in G1 + G2:
            g.start()
        for c in range(NC):
            for b in range(B):
                gp[b, c, pl.ds(0, ZP), :] = jnp.zeros((ZP, 128), f32)
            gm[c, pl.ds(CARRY + T - P, ZP), :] = jnp.zeros((ZP, 128), f32)

        for g in G1:
            g.wait()
        for g in G3 + [xm(0), xm(1)]:
            g.start()
        xv = arena[pl.ds(0, P), pl.ds(0, KH)]
        for half in range(2):
            base = W1B if half else W1A
            hp[half] = jnp.dot(xv, arena[pl.ds(base, KH), :], preferred_element_type=f32)

        for g in G2:
            g.wait()
        g0 = gp.at[0]
        for s in range(len(pt) + 1):
            if s < len(pt):
                lo, hi = pt[s]
                xv = arena[pl.ds(lo, hi - lo), pl.ds(KH, KH)]
                for c2 in range(NC // 2):
                    cols = pl.ds(c2 * 256, 256)
                    a = hp[0, pl.ds(lo, hi - lo), cols] + jnp.dot(xv, arena[pl.ds(W1A + KH, KH), cols], preferred_element_type=f32)
                    b = hp[1, pl.ds(lo, hi - lo), cols] + jnp.dot(xv, arena[pl.ds(W1B + KH, KH), cols], preferred_element_type=f32)
                    gv = glu(a, b)
                    g0[2 * c2, pl.ds(ZP + lo, hi - lo), :] = gv[:, :128]
                    g0[2 * c2 + 1, pl.ds(ZP + lo, hi - lo), :] = gv[:, 128:]
            if s >= 1:
                lo, hi = pb[s - 1]
                conv_mm2(g0, ZP + lo, hi - lo, lo)

        for g in G3:
            g.wait()
        g1 = gp.at[1]
        for s in range(len(pt) + 1):
            if s < len(pt):
                lo, hi = pt[s]
                mm1(arena[pl.ds(T + lo, hi - lo), :], g1, ZP + lo)
            if s >= 1:
                lo, hi = pb[s - 1]
                conv_mm2(g1, ZP + lo, hi - lo, T + lo)

        def main(bi, carry):
            base = pl.multiple_of(bi * T, 16)
            cp(x_hbm.at[pl.ds(base + P, T - P), :], arena.at[pl.ds(base + P, T - P), :], sem.at[3 + bi]).wait()
            for c in range(NC):
                gm[c, pl.ds(0, CARRY), :] = gp[bi, c, pl.ds(ZP + P - CARRY, CARRY), :]
            nt = len(mt)
            for s in range(nt + 1):
                if s < nt:
                    lo, hi = mt[s]
                    mm1(arena[pl.ds(base + lo, hi - lo), :], gm, lo - P + CARRY)
                if s >= 1:
                    lo, hi = mb[s - 1]
                    conv_mm2(gm, lo - P + CARRY, hi - lo, base + lo)
            return carry

        lax.fori_loop(0, B, main, 0)
        ocopy(0, R).wait()

    out = pl.pallas_call(
        body,
        in_specs=[pl.BlockSpec(memory_space=pl.ANY)] * 4,
        out_specs=pl.BlockSpec(memory_space=pl.ANY),
        out_shape=jax.ShapeDtypeStruct((R, D), x.dtype),
        scratch_shapes=[
            pltpu.VMEM((AR, D), bf16),
            pltpu.VMEM((R, D), bf16),
            pltpu.VMEM((2, P, D), f32),
            pltpu.VMEM((B, NC, ZP + P, 128), f32),
            pltpu.VMEM((NC, CARRY + T - P + ZP, 128), f32),
            pltpu.VMEM((K, D), bf16),
            pltpu.SemaphoreType.DMA((6,)),
        ],
        compiler_params=pltpu.CompilerParams(vmem_limit_bytes=100 * 1024 * 1024),
    )(x2, w_pw1, dw, w_pw2)
    return out.reshape(B, T, D)
```

```python
import jax
import jax.numpy as jnp
from jax import lax
import jax.experimental.pallas as pl
import jax.experimental.pallas.tpu as pltpu

P = 640
HS = 400
TAIL = (256, 128)
KS = (128, 128, 256)
NCOLFLUSH = 2
LAG = 16
ZP = 8
CARRY = 24


def _split(lo, hi, hs, tail=()):
    out = []
    r = lo
    body_end = hi - sum(tail)
    n_tiles = max(1, round((body_end - lo) / hs))
    assert (body_end - lo) % 16 == 0
    units = (body_end - lo) // 16
    for i in range(n_tiles):
        u = units // n_tiles + (1 if i < units % n_tiles else 0)
        out.append((r, r + 16 * u))
        r += 16 * u
    for n in tail:
        out.append((r, r + n))
        r += n
    assert r == hi
    return out


@jax.jit
def pallas_standalone__conformer_conv_module__speech_kernel(
    x: jax.Array,
    w_pw1: jax.Array,
    dw: jax.Array,
    w_pw2: jax.Array,
):
    B, T, D = x.shape
    K = dw.shape[0]
    PAD = K // 2
    NC = D // 128
    R = B * T
    f32 = jnp.float32
    bf16 = jnp.bfloat16
    assert B == 2 and sum(KS) == D and T % 16 == 0 and PAD < ZP and K <= 16
    assert LAG + PAD <= CARRY and PAD <= LAG

    mt = _split(P, T, HS, TAIL)
    mb = [(lo - LAG, hi - LAG if hi < T else T) for lo, hi in mt]
    pt = _split(0, P, P // 2)
    pb = [(max(lo - LAG, 0), hi - LAG) for lo, hi in pt]
    n_st = len(KS)
    W2 = R

    def body(x_hbm, w1_hbm, dw_hbm, w2_hbm, o_hbm,
             arena, obuf, hp, gp, gm, dwbuf, w1raw, w1n, w2n, sem):
        cp = pltpu.make_async_copy

        stage_cp = []
        k0 = 0
        for i, kk in enumerate(KS):
            stage_cp.append([
                cp(w1_hbm.at[pl.ds(k0, kk), :], w1raw.at[pl.ds(k0, kk), :], sem.at[i]),
                cp(x_hbm.at[pl.ds(0, P), pl.ds(k0, kk)],
                   arena.at[pl.ds(0, P), pl.ds(k0, kk)], sem.at[i]),
            ])
            k0 += kk
        rest_cp = [
            cp(x_hbm.at[pl.ds(T, P), :], arena.at[pl.ds(T, P), :], sem.at[n_st]),
            cp(dw_hbm, dwbuf, sem.at[n_st]),
            cp(w2_hbm, arena.at[pl.ds(W2, D), :], sem.at[n_st]),
        ]

        def x_main(b, row):
            return cp(x_hbm.at[pl.ds(row, T - P), :], arena.at[pl.ds(row, T - P), :],
                      sem.at[n_st + 1 + b])

        def out_cp(row, n, col=0, ncol=D):
            return cp(obuf.at[pl.ds(row, n), pl.ds(col, ncol)],
                      o_hbm.at[pl.ds(row, n), pl.ds(col, ncol)], sem.at[n_st + 3])

        def glu(a, half_b):
            return a * (jnp.tanh(half_b) + 1.0)

        def mm1(xv, gref, grow, hook=None):
            n = xv.shape[0]
            for c in range(NC):
                if hook is not None:
                    hook(c)
                wa = pltpu.bitcast(w1n[:, c * 128:(c + 1) * 128], bf16)
                wb = pltpu.bitcast(w1n[:, D + c * 128:D + (c + 1) * 128], bf16)
                a = jnp.dot(xv, wa, preferred_element_type=f32)
                hb = jnp.dot(xv, wb, preferred_element_type=f32)
                gref[c, pl.ds(grow, n), :] = glu(a, hb)

        def taps_vpu(c):
            return dwbuf[:, c * 128:(c + 1) * 128].astype(f32) * 0.25

        def taps_mxu(c):
            r = lax.broadcasted_iota(jnp.int32, (16, K), 0)
            q = lax.broadcasted_iota(jnp.int32, (16, K), 1)
            eye = jnp.where(r == q, 0.25, 0.0).astype(bf16)
            return jnp.dot(eye, dwbuf[:, c * 128:(c + 1) * 128], preferred_element_type=f32)

        def conv_silu(gref, grow, n, c, taps):
            acc = None
            for i in range(K):
                term = gref[c, pl.ds(grow - PAD + i, n), :] * taps[i:i + 1, :]
                acc = term if acc is None else acc + term
            return acc * (jnp.tanh(acc) + 1.0)

        def conv_mm2(gref, grow, n, orow, taps=None, colflush=False):
            sv = jnp.concatenate(
                [conv_silu(gref, grow, n, c, taps_vpu(c) if taps is None else taps[c])
                 for c in range(NC)], axis=1).astype(bf16)
            cw = 128 if colflush else D
            for col in range(0, D, cw):
                w = pltpu.bitcast(w2n[:, col:col + cw], bf16)
                obuf[pl.ds(orow, n), pl.ds(col, cw)] = jnp.dot(
                    sv, w, preferred_element_type=f32).astype(bf16)
                out_cp(orow, n, col, cw).start()

        def prologue():
            g0 = gp.at[0]
            k0 = 0
            for i, kk in enumerate(KS):
                for c_ in stage_cp[i]:
                    c_.wait()
                if i == 0:
                    x_main(0, P).start()
                    x_main(1, T + P).start()
                xv = arena[pl.ds(0, P), pl.ds(k0, kk)]
                wa = w1raw[pl.ds(k0, kk), pl.ds(0, D)]
                wb = (w1raw[pl.ds(k0, kk), pl.ds(D, D)].astype(f32) * 0.5).astype(bf16)
                if i < n_st - 1:
                    for half, w in enumerate((wa, wb)):
                        part = jnp.dot(xv, w, preferred_element_type=f32)
                        hp[half] = part if i == 0 else hp[half] + part
                else:
                    for c2 in range(NC // 2):
                        lo, hi = c2 * 256, (c2 + 1) * 256
                        a = hp[0, :, lo:hi] + jnp.dot(xv, wa[:, lo:hi], preferred_element_type=f32)
                        hb = hp[1, :, lo:hi] + jnp.dot(xv, wb[:, lo:hi], preferred_element_type=f32)
                        gv = glu(a, hb)
                        g0[2 * c2, pl.ds(ZP, P), :] = gv[:, :128]
                        g0[2 * c2 + 1, pl.ds(ZP, P), :] = gv[:, 128:]
                w1n[pl.ds(k0 // 2, kk // 2), pl.ds(0, D)] = pltpu.bitcast(wa, jnp.uint32)
                w1n[pl.ds(k0 // 2, kk // 2), pl.ds(D, D)] = pltpu.bitcast(wb, jnp.uint32)
                k0 += kk

            for c_ in rest_cp:
                c_.wait()
            w2n[...] = pltpu.bitcast(arena[pl.ds(W2, D), :], jnp.uint32)
            taps = {}
            g1 = gp.at[1]

            def hook(c):
                taps[c] = taps_mxu(c)

            for s, (lo, hi) in enumerate(pt):
                mm1(arena[pl.ds(T + lo, hi - lo), :], g1, ZP + lo, hook if s == 0 else None)
            conv_mm2(g0, ZP, P - LAG, 0, taps)
            for lo, hi in pb:
                conv_mm2(g1, ZP + lo, hi - lo, T + lo)

        def main(bi, carry):
            pl.when(bi == 0)(prologue)
            base = pl.multiple_of(bi * T, 16)
            x_main(bi, base + P).wait()
            for c in range(NC):
                gm[c, pl.ds(0, CARRY), :] = gp[bi, c, pl.ds(ZP + P - CARRY, CARRY), :]
            nt = len(mt)
            for s in range(nt + 1):
                if s < nt:
                    lo, hi = mt[s]
                    mm1(arena[pl.ds(base + lo, hi - lo), :], gm, lo - P + CARRY)
                if s >= 1:
                    lo, hi = mb[s - 1]
                    conv_mm2(gm, lo - P + CARRY, hi - lo, base + lo,
                             colflush=s > nt - NCOLFLUSH)
            return carry

        for c_ in stage_cp[0] + stage_cp[1] + stage_cp[2] + rest_cp:
            c_.start()
        zeros = jnp.zeros((ZP, 128), f32)
        for c in range(NC):
            for b in range(B):
                gp[b, c, pl.ds(0, ZP), :] = zeros
            gm[c, pl.ds(CARRY + T - P, ZP), :] = zeros
        lax.fori_loop(0, B, main, 0)
        out_cp(0, R).wait()

    out = pl.pallas_call(
        body,
        in_specs=[pl.BlockSpec(memory_space=pl.ANY)] * 4,
        out_specs=pl.BlockSpec(memory_space=pl.ANY),
        out_shape=jax.ShapeDtypeStruct((R, D), x.dtype),
        scratch_shapes=[
            pltpu.VMEM((R + D, D), bf16),
            pltpu.VMEM((R, D), bf16),
            pltpu.VMEM((2, P, D), f32),
            pltpu.VMEM((B, NC, ZP + P, 128), f32),
            pltpu.VMEM((NC, CARRY + T - P + ZP, 128), f32),
            pltpu.VMEM((K, D), bf16),
            pltpu.VMEM((D, 2 * D), bf16),
            pltpu.VMEM((D // 2, 2 * D), jnp.uint32),
            pltpu.VMEM((D // 2, D), jnp.uint32),
            pltpu.SemaphoreType.DMA((n_st + 4,)),
        ],
        compiler_params=pltpu.CompilerParams(
            vmem_limit_bytes=64 * 1024 * 1024,
            disable_bounds_checks=True,
            disable_semaphore_checks=True,
        ),
    )(x.reshape(R, D), w_pw1, dw, w_pw2)
    return out.reshape(B, T, D)
```

```python
import jax
import jax.numpy as jnp
from jax import lax
import jax.experimental.pallas as pl
import jax.experimental.pallas.tpu as pltpu

P = 640
HS = 400
TAIL = (256, 128)
KS = (128, 128, 256)
N1 = 480
NCOLFLUSH = 2
LAG = 16
ZP = 8
CARRY = 24


def _split(lo, hi, hs, tail=()):
    out = []
    r = lo
    body_end = hi - sum(tail)
    n_tiles = max(1, round((body_end - lo) / hs))
    assert (body_end - lo) % 16 == 0
    units = (body_end - lo) // 16
    for i in range(n_tiles):
        u = units // n_tiles + (1 if i < units % n_tiles else 0)
        out.append((r, r + 16 * u))
        r += 16 * u
    for n in tail:
        out.append((r, r + n))
        r += n
    assert r == hi
    return out


@jax.jit
def pallas_standalone__conformer_conv_module__speech_kernel(
    x: jax.Array,
    w_pw1: jax.Array,
    dw: jax.Array,
    w_pw2: jax.Array,
):
    B, T, D = x.shape
    K = dw.shape[0]
    PAD = K // 2
    NC = D // 128
    R = B * T
    f32 = jnp.float32
    bf16 = jnp.bfloat16
    assert B == 2 and sum(KS) == D and T % 16 == 0 and PAD < ZP and K <= 16
    assert LAG + PAD <= CARRY and PAD <= LAG

    mt = _split(P, T, HS, TAIL)
    mb = [(lo - LAG, hi - LAG if hi < T else T) for lo, hi in mt]
    pt = _split(0, P, P // 2)
    pb = [(max(lo - LAG, 0), hi - LAG) for lo, hi in pt]
    n_st = len(KS)
    W2 = R

    def body(x_hbm, w1_hbm, dw_hbm, w2_hbm, o_hbm,
             arena, obuf, hp, gp, gm, dwbuf, w1raw, w1n, w2n, sem):
        cp = pltpu.make_async_copy

        stage_cp = []
        k0 = 0
        for i, kk in enumerate(KS):
            rows = N1 if i == 0 else P
            stage_cp.append([
                cp(w1_hbm.at[pl.ds(k0, kk), :], w1raw.at[pl.ds(k0, kk), :], sem.at[i]),
                cp(x_hbm.at[pl.ds(0, rows), pl.ds(k0, kk)],
                   arena.at[pl.ds(0, rows), pl.ds(k0, kk)], sem.at[i]),
            ])
            if i == 1 and N1 < P:
                stage_cp[1].append(
                    cp(x_hbm.at[pl.ds(N1, P - N1), pl.ds(0, KS[0])],
                       arena.at[pl.ds(N1, P - N1), pl.ds(0, KS[0])], sem.at[1]))
            k0 += kk
        rest_cp = [
            cp(x_hbm.at[pl.ds(T, P), :], arena.at[pl.ds(T, P), :], sem.at[n_st]),
            cp(dw_hbm, dwbuf, sem.at[n_st]),
            cp(w2_hbm, arena.at[pl.ds(W2, D), :], sem.at[n_st]),
        ]

        def x_main(b, row):
            return cp(x_hbm.at[pl.ds(row, T - P), :], arena.at[pl.ds(row, T - P), :],
                      sem.at[n_st + 1 + b])

        def out_cp(row, n, col=0, ncol=D):
            return cp(obuf.at[pl.ds(row, n), pl.ds(col, ncol)],
                      o_hbm.at[pl.ds(row, n), pl.ds(col, ncol)], sem.at[n_st + 3])

        def glu(a, half_b):
            return a * (jnp.tanh(half_b) + 1.0)

        def mm1(xv, gref, grow, hook=None):
            n = xv.shape[0]
            for c in range(NC):
                if hook is not None:
                    hook(c)
                wa = pltpu.bitcast(w1n[:, c * 128:(c + 1) * 128], bf16)
                wb = pltpu.bitcast(w1n[:, D + c * 128:D + (c + 1) * 128], bf16)
                a = jnp.dot(xv, wa, preferred_element_type=f32)
                hb = jnp.dot(xv, wb, preferred_element_type=f32)
                gref[c, pl.ds(grow, n), :] = glu(a, hb)

        def taps_vpu(c):
            return dwbuf[:, c * 128:(c + 1) * 128].astype(f32) * 0.25

        def taps_mxu(c):
            r = lax.broadcasted_iota(jnp.int32, (16, K), 0)
            q = lax.broadcasted_iota(jnp.int32, (16, K), 1)
            eye = jnp.where(r == q, 0.25, 0.0).astype(bf16)
            return jnp.dot(eye, dwbuf[:, c * 128:(c + 1) * 128], preferred_element_type=f32)

        def conv_silu(gref, grow, n, c, taps):
            acc = None
            for i in range(K):
                term = gref[c, pl.ds(grow - PAD + i, n), :] * taps[i:i + 1, :]
                acc = term if acc is None else acc + term
            return acc * (jnp.tanh(acc) + 1.0)

        def conv_mm2(gref, grow, n, orow, taps=None, colflush=False):
            sv = jnp.concatenate(
                [conv_silu(gref, grow, n, c, taps_vpu(c) if taps is None else taps[c])
                 for c in range(NC)], axis=1).astype(bf16)
            cw = 128 if colflush else D
            for col in range(0, D, cw):
                w = pltpu.bitcast(w2n[:, col:col + cw], bf16)
                obuf[pl.ds(orow, n), pl.ds(col, cw)] = jnp.dot(
                    sv, w, preferred_element_type=f32).astype(bf16)
                out_cp(orow, n, col, cw).start()

        def prologue():
            g0 = gp.at[0]
            k0 = 0
            for i, kk in enumerate(KS):
                for c_ in stage_cp[i]:
                    c_.wait()
                if i == 0:
                    x_main(0, P).start()
                    x_main(1, T + P).start()
                xv = arena[pl.ds(0, N1 if i == 0 else P), pl.ds(k0, kk)]
                wa = w1raw[pl.ds(k0, kk), pl.ds(0, D)]
                wb = (w1raw[pl.ds(k0, kk), pl.ds(D, D)].astype(f32) * 0.5).astype(bf16)
                if i == 1 and N1 < P:
                    xr = arena[pl.ds(N1, P - N1), pl.ds(0, KS[0])]
                    for half in range(2):
                        w0 = pltpu.bitcast(w1n[pl.ds(0, KS[0] // 2), pl.ds(half * D, D)], bf16)
                        hp[half, pl.ds(N1, P - N1), :] = jnp.dot(xr, w0, preferred_element_type=f32)
                if i < n_st - 1:
                    for half, w in enumerate((wa, wb)):
                        part = jnp.dot(xv, w, preferred_element_type=f32)
                        if i == 0:
                            hp[half, pl.ds(0, N1), :] = part
                        else:
                            hp[half] = hp[half] + part
                else:
                    for c2 in range(NC // 2):
                        lo, hi = c2 * 256, (c2 + 1) * 256
                        a = hp[0, :, lo:hi] + jnp.dot(xv, wa[:, lo:hi], preferred_element_type=f32)
                        hb = hp[1, :, lo:hi] + jnp.dot(xv, wb[:, lo:hi], preferred_element_type=f32)
                        gv = glu(a, hb)
                        g0[2 * c2, pl.ds(ZP, P), :] = gv[:, :128]
                        g0[2 * c2 + 1, pl.ds(ZP, P), :] = gv[:, 128:]
                w1n[pl.ds(k0 // 2, kk // 2), pl.ds(0, D)] = pltpu.bitcast(wa, jnp.uint32)
                w1n[pl.ds(k0 // 2, kk // 2), pl.ds(D, D)] = pltpu.bitcast(wb, jnp.uint32)
                k0 += kk

            for c_ in rest_cp:
                c_.wait()
            w2n[...] = pltpu.bitcast(arena[pl.ds(W2, D), :], jnp.uint32)
            taps = {}
            g1 = gp.at[1]

            def hook(c):
                taps[c] = taps_mxu(c)

            for s, (lo, hi) in enumerate(pt):
                mm1(arena[pl.ds(T + lo, hi - lo), :], g1, ZP + lo, hook if s == 0 else None)
            conv_mm2(g0, ZP, P - LAG, 0, taps)
            for lo, hi in pb:
                conv_mm2(g1, ZP + lo, hi - lo, T + lo)

        def main(bi, carry):
            pl.when(bi == 0)(prologue)
            base = pl.multiple_of(bi * T, 16)
            x_main(bi, base + P).wait()
            for c in range(NC):
                gm[c, pl.ds(0, CARRY), :] = gp[bi, c, pl.ds(ZP + P - CARRY, CARRY), :]
            nt = len(mt)
            for s in range(nt + 1):
                if s < nt:
                    lo, hi = mt[s]
                    mm1(arena[pl.ds(base + lo, hi - lo), :], gm, lo - P + CARRY)
                if s >= 1:
                    lo, hi = mb[s - 1]
                    conv_mm2(gm, lo - P + CARRY, hi - lo, base + lo,
                             colflush=s > nt - NCOLFLUSH)
            return carry

        for c_ in stage_cp[0] + stage_cp[1] + stage_cp[2] + rest_cp:
            c_.start()
        zeros = jnp.zeros((ZP, 128), f32)
        for c in range(NC):
            for b in range(B):
                gp[b, c, pl.ds(0, ZP), :] = zeros
            gm[c, pl.ds(CARRY + T - P, ZP), :] = zeros
        lax.fori_loop(0, B, main, 0)
        out_cp(0, R).wait()

    out = pl.pallas_call(
        body,
        in_specs=[pl.BlockSpec(memory_space=pl.ANY)] * 4,
        out_specs=pl.BlockSpec(memory_space=pl.ANY),
        out_shape=jax.ShapeDtypeStruct((R, D), x.dtype),
        scratch_shapes=[
            pltpu.VMEM((R + D, D), bf16),
            pltpu.VMEM((R, D), bf16),
            pltpu.VMEM((2, P, D), f32),
            pltpu.VMEM((B, NC, ZP + P, 128), f32),
            pltpu.VMEM((NC, CARRY + T - P + ZP, 128), f32),
            pltpu.VMEM((K, D), bf16),
            pltpu.VMEM((D, 2 * D), bf16),
            pltpu.VMEM((D // 2, 2 * D), jnp.uint32),
            pltpu.VMEM((D // 2, D), jnp.uint32),
            pltpu.SemaphoreType.DMA((n_st + 4,)),
        ],
        compiler_params=pltpu.CompilerParams(
            vmem_limit_bytes=64 * 1024 * 1024,
            disable_bounds_checks=True,
            disable_semaphore_checks=True,
        ),
    )(x.reshape(R, D), w_pw1, dw, w_pw2)
    return out.reshape(B, T, D)
```
